```python
import os as _os
_os.environ.setdefault("JAX_PLATFORMS", "cpu")
import jax
import jax.numpy as jnp

def _softmax(x, axis=-1):
    return jax.nn.softmax(x, axis=axis)
def _gelu(x):
    return jax.nn.gelu(x, approximate=True)
def _silu(x):
    return jax.nn.silu(x)
def _sigmoid(x):
    return jax.nn.sigmoid(x)
def _layernorm(x, axis=-1, eps=1e-5):
    m = jnp.mean(x, axis=axis, keepdims=True)
    v = jnp.var(x, axis=axis, keepdims=True)
    return (x - m) / jnp.sqrt(v + eps)
def _scatter_add(tgt, idx, src, axis=0):
    return tgt.at[idx].add(src)
def _segment_sum(src, seg, n):
    return jax.ops.segment_sum(src, seg, n)
class _Rng:
    def __init__(self, key):
        self._k = key
    def _next(self):
        self._k, sub = jax.random.split(self._k)
        return sub
    def normal(self, shape):
        return jax.random.normal(self._next(), shape, dtype=jnp.bfloat16)
    def randint(self, lo, hi, shape):
        return jax.random.randint(self._next(), shape, lo, hi, dtype=jnp.int32)
    def uniform(self, shape, lo=0.0, hi=1.0):
        return jax.random.uniform(self._next(), shape, jnp.bfloat16, lo, hi)
    def permutation(self, n):
        return jax.random.permutation(self._next(), n)


kernel_name = 'concat_heads__ssm_conv_h3__sliding_block__prompt'

def setup_inputs():
    _rng = _Rng(jax.random.key(int.from_bytes(__import__("os").urandom(4), "little")))
    _w = (lambda a: (lambda t: t.astype(jnp.bfloat16) if jnp.issubdtype(t.dtype, jnp.floating) else t)(jnp.asarray(a)))
    def _A_setup():
        B, S, D = 1, 2048, 512
        ks = 4
        return {
            "q": _w((lambda *s: _rng.normal(s) * 0.05)(B, S, D)),
            "k": _w((lambda *s: _rng.normal(s) * 0.2)(B, S, D)),
            "v": _w((lambda *s: _rng.normal(s) * 0.2)(B, S, D)),
            "shift_k": _w((lambda *s: _rng.normal(s) * 0.2)(D, ks) * 0.5),
            "ssm_k": _w((lambda *s: _rng.normal(s) * 0.2)(D, S) * (1.0 / S ** 0.5)),
            "ssm_D": _w((lambda *s: _rng.normal(s) * 0.2)(D)),
        }
    _A_in = _A_setup()

    def _B_setup():
        B, S, D = 1, 2048, 512
        return {
            "x": _w((lambda *s: _rng.normal(s) * 0.2)(B, S, D)),
            "wqkv": _w((lambda *s: _rng.normal(s) * 0.2)(D, 3 * D)),
            "wo": _w((lambda *s: _rng.normal(s) * 0.05)(D, D)),
        }
    _B_in = _B_setup()

    return {
        "A_q": _A_in["q"],
        "A_k": _A_in["k"],
        "A_v": _A_in["v"],
        "A_shift_k": _A_in["shift_k"],
        "A_ssm_k": _A_in["ssm_k"],
        "A_ssm_D": _A_in["ssm_D"],
        "B_x": _B_in["x"],
        "B_wqkv": _B_in["wqkv"],
        "B_wo": _B_in["wo"],
    }

def reference(A_q, A_k, A_v, A_shift_k, A_ssm_k, A_ssm_D, B_x, B_wqkv, B_wo):
    def _A_ref(q, k, v, shift_k, ssm_k, ssm_D):
        B, S, D = q.shape
        ks = shift_k.shape[-1]
        k_pad = jnp.pad(k, ((0, 0), (ks - 1, 0), (0, 0)))
        k_shift = jnp.zeros_like(k)
        for t in range(ks):
            k_shift = k_shift + k_pad[:, t:t + S, :] * shift_k[:, ks - 1 - t][None, None, :]
        kv = k_shift * v
        L = 2 * S
        kv_pad = jnp.pad(kv, ((0, 0), (0, S), (0, 0)))
        kf_pad = jnp.pad(ssm_k, ((0, 0), (0, S)))
        kv_f = (lambda x, axes=(-2,-1): jnp.fft.rfft2(x.astype(jnp.float32), axes=axes))(kv_pad[:, None, :, :], axes=(1, 2))
        kf_f = (lambda x, axes=(-2,-1): jnp.fft.rfft2(x.astype(jnp.float32), axes=axes))(kf_pad[:, None, :], axes=(1, 2))
        kf_f = (lambda x, *d: x.transpose(*d))(kf_f, 1, 2, 0)
        y_f = kv_f * kf_f[None, :, :, :]
        y = (lambda x, s, axes=(-2,-1): jnp.fft.irfft2(x, s=s, axes=axes).astype(jnp.bfloat16))(y_f, (1, L), axes=(1, 2))[:, 0, :S, :]
        y = y + kv * ssm_D[None, None, :]
        return q * y

    def _B_ref(x, wqkv, wo):
        B, S, D = x.shape
        H = 32; Dh = D // H; W = 256
        qkv = (lambda x, *d: x.transpose(*d))((x @ wqkv).reshape(B, S, 3, H, Dh), 2, 0, 3, 1, 4)
        q, k, v = qkv[0], qkv[1], qkv[2]
        scores = jnp.einsum("bhqd,bhkd->bhqk", q, k) * (Dh ** -0.5)
        idx = jnp.arange(S)
        mask = (idx[:, None] - idx[None, :] >= 0) & (idx[:, None] - idx[None, :] < W)
        scores = jnp.where(mask[None, None], scores, -1e9)
        p = _softmax(scores, axis=-1)
        o = jnp.einsum("bhqk,bhkd->bhqd", p, v)
        return (lambda x, *d: x.transpose(*d))(o, 0, 2, 1, 3).reshape(B, S, D) @ wo

    a = _A_ref(A_q, A_k, A_v, A_shift_k, A_ssm_k, A_ssm_D)
    b = _B_ref(B_x, B_wqkv, B_wo)
    return jnp.concatenate([a, b], axis=-1)
```

```python
import math

import numpy as np
import jax
import jax.numpy as jnp
from jax import lax
import jax.experimental.pallas as pl
import jax.experimental.pallas.tpu as pltpu

S, D = 2048, 512
H, DH, W = 32, 16, 256
C = 128
NC = S // C
BS = 256
NS = S // BS
NEG = -1e30
NT = (((1,), (1,)), ((), ()))
TN = (((0,), (0,)), ((), ()))
f32, bf16 = jnp.float32, jnp.bfloat16


def _consts():
    th = 2 * np.pi * np.outer(np.arange(C) + 0.5, np.arange(C)) / (2 * C)
    fwd = np.concatenate([np.cos(th), -np.sin(th)], 0)
    inv = np.concatenate([np.cos(th).T, -np.sin(th).T], 1) / C
    return fwd.astype(np.float32), inv.astype(np.float32)


def _kernel(aq_ref, ak_ref, av_ref, sh_ref, h_ref, dd_ref, x_ref, wqkv_ref, wo_ref,
            fwd_ref, inv_ref, o_ref,
            wvt, qs, ks, vts, ots, bias, kbuf, kvs, us, hs, hprev, zs,
            sa, ma, sb_, mb_):
    step = pl.program_id(0)

    @pl.when(step == 0)
    def _init():
        wvt[...] = wqkv_ref[:, 2 * D:].astype(f32).T.astype(bf16)
        ks[:, 0:2] = jnp.zeros((4, 2, 128, 128), bf16)
        vts[...] = jnp.ones(vts.shape, bf16)
        vts[0:2] = jnp.zeros((2,) + vts.shape[1:], bf16)
        kbuf[0:8, :] = jnp.zeros((8, D), f32)
        hprev[...] = jnp.zeros(hprev.shape, f32)
        r = lax.broadcasted_iota(jnp.int32, (128, 128), 0)
        c = lax.broadcasted_iota(jnp.int32, (128, 128), 1)
        bias[0] = jnp.full((128, 128), NEG, f32)
        bias[1] = jnp.where(r > c, 0.0, NEG)
        bias[2] = jnp.where(r <= c, 0.0, NEG)

    @pl.when(step < NS)
    def _phase1():
        s = step
        x = x_ref[...]
        qk = jnp.dot(x, wqkv_ref[:, :2 * D], preferred_element_type=f32)
        q = (qk[:, :D] * (DH ** -0.5 * math.log2(math.e))).astype(bf16)
        k = qk[:, D:].astype(bf16)
        row = pl.multiple_of(s * BS, BS)
        for g in range(4):
            for t in range(2):
                qs[g, 2 * s + t] = q[128 * t:128 * t + 128, g * 128:(g + 1) * 128]
                ks[g, 2 + 2 * s + t] = k[128 * t:128 * t + 128, g * 128:(g + 1) * 128]
        vt = lax.dot_general(wvt[...], x, NT, preferred_element_type=f32).astype(bf16)
        for t in range(2):
            for h in range(H):
                vts[2 + 2 * s + t, h // 8, 32 * (h % 8):32 * (h % 8) + 16, :] = (
                    vt[16 * h:16 * h + 16, 128 * t:128 * t + 128])

        kbuf[8:, :] = ak_ref[...].astype(f32)
        sh = sh_ref[...].astype(f32)
        acc = kbuf[8:8 + BS, :] * sh[0:1]
        for t in range(1, 4):
            acc = acc + kbuf[8 - t:8 - t + BS, :] * sh[t:t + 1]
        kv = (acc * av_ref[...].astype(f32)).astype(bf16)
        kbuf[0:8, :] = kbuf[BS:BS + 8, :]
        kvs[pl.ds(row, BS), :] = kv
        fwd = fwd_ref[...]
        sg = (1 - 2 * (lax.broadcasted_iota(jnp.int32, (C, D), 0) & 1)).astype(f32)
        for t in range(2):
            u = jnp.dot(fwd, kv[C * t:C * t + C], preferred_element_type=f32)
            hf = lax.dot_general(fwd, h_ref[:, C * t:C * t + C], NT,
                                 preferred_element_type=f32)
            hr = hf[:C] - sg * hprev[C:, :]
            hi = hf[C:] + sg * hprev[:C, :]
            hprev[...] = hf
            for g in range(4):
                ls = slice(g * 128, (g + 1) * 128)
                us[g, 2 * s + t] = u[:, ls]
                hs[g, 2 * s + t, :C, :] = hr[:, ls]
                hs[g, 2 * s + t, C:, :] = hi[:, ls]

    lane_head = lax.broadcasted_iota(jnp.int32, (64, 128), 1) // DH

    def scores(it, h0, sb, mb):
        g = it % 4
        tile = it // 4
        b0 = jnp.where(tile >= 2, 1, 0)
        b1 = jnp.where(tile >= 1, 0.0, NEG)
        qt = pltpu.bitcast(qs[g, tile], jnp.int32)
        kw = jnp.concatenate([ks[g, tile + j] for j in range(3)], axis=0)
        for n in range(4):
            qm = pltpu.bitcast(jnp.where(lane_head == h0 + n, qt, 0), bf16)
            sc = lax.dot_general(kw, qm, NT, preferred_element_type=f32)
            s0 = sc[:128] + bias[b0]
            s1 = sc[128:256] + b1
            s2 = sc[256:] + bias[2]
            sb[n, 0:128] = s0
            sb[n, 128:256] = s1
            sb[n, 256:384] = s2
            m = jnp.maximum(jnp.maximum(s0, s1), s2).reshape(16, 8, 128).max(axis=0)
            mb[n] = jnp.broadcast_to(jnp.max(m, axis=0, keepdims=True), (8, 128))

    def attend(it, h0, sb, mb):
        g = it % 4
        tile = it // 4
        for n in range(4):
            hh = h0 + n
            p = jnp.exp2(sb[n] - jnp.concatenate([mb[n]] * 48, axis=0))
            ot = None
            for j in range(3):
                d = jnp.dot(vts[tile + j, g, 32 * hh:32 * hh + 32, :],
                            p[128 * j:128 * j + 128].astype(bf16), preferred_element_type=f32)
                ot = d if ot is None else ot + d
            ots[tile, g, 16 * hh:16 * hh + 16, :] = (ot[:16] / ot[16:]).astype(bf16)

    def conv(it, i):
        g = it % 4
        fr = pl.multiple_of((it // 4) * 8, 8)
        zr = zi = None
        for m_ in range(i + 1):
            hr = hs[g, m_, pl.ds(fr, 8), :]
            hi = hs[g, m_, pl.ds(fr + C, 8), :]
            ur = us[g, i - m_, pl.ds(fr, 8), :]
            ui = us[g, i - m_, pl.ds(fr + C, 8), :]
            a = hr * ur - hi * ui
            b = hr * ui + hi * ur
            zr = a if zr is None else zr + a
            zi = b if zi is None else zi + b
        zs[g, i, pl.ds(fr, 8), :] = zr
        zs[g, i, pl.ds(fr + C, 8), :] = zi

    @pl.when(step == NS)
    def _():
        scores(0, 0, sa, ma)

    @pl.when((step >= NS) & (step < 2 * NS))
    def _phase2():
        def body(j, _):
            it = (step - NS) * 8 + j
            scores(it, 4, sb_, mb_)
            attend(it, 0, sa, ma)
            for i in range(4):
                conv(it, i)
                conv(it, NC - 1 - i)
            scores(jnp.minimum(it + 1, 63), 0, sa, ma)
            attend(it, 4, sb_, mb_)
            for i in range(4, 8):
                conv(it, i)
                conv(it, NC - 1 - i)
            return 0

        lax.fori_loop(0, 8, body, 0)

    @pl.when(step >= 2 * NS)
    def _phase3():
        s = step - 2 * NS
        row = pl.multiple_of(s * BS, BS)
        inv = inv_ref[...]
        dd = dd_ref[...].astype(f32)
        for t in range(2):
            rs = slice(C * t, C * t + C)
            o_ref[rs, D:] = lax.dot_general(
                ots[2 * s + t].reshape(D, 128), wo_ref[...], TN, preferred_element_type=f32).astype(bf16)
            for g in range(4):
                ls = slice(g * 128, (g + 1) * 128)
                y = jnp.dot(inv, zs[g, 2 * s + t].astype(bf16), preferred_element_type=f32)
                kv = kvs[pl.ds(row + C * t, C), ls].astype(f32)
                y = y + kv * dd[:, ls]
                o_ref[rs, ls] = (aq_ref[rs, ls].astype(f32) * y).astype(bf16)


@jax.jit
def pallas_concat_heads__ssm_conv_h3__sliding_block__prompt_kernel(
    A_q: jax.Array,
    A_k: jax.Array,
    A_v: jax.Array,
    A_shift_k: jax.Array,
    A_ssm_k: jax.Array,
    A_ssm_D: jax.Array,
    B_x: jax.Array,
    B_wqkv: jax.Array,
    B_wo: jax.Array,
):
    fwd, inv = _consts()
    p1 = lambda i: (jnp.minimum(i, NS - 1), 0)
    p3 = lambda i: (jnp.maximum(i - 2 * NS, 0), 0)
    fixed = lambda i: (0, 0)
    out = pl.pallas_call(
        _kernel,
        grid=(3 * NS,),
        in_specs=[
            pl.BlockSpec((BS, D), p3),
            pl.BlockSpec((BS, D), p1),
            pl.BlockSpec((BS, D), p1),
            pl.BlockSpec((4, D), fixed),
            pl.BlockSpec((D, BS), lambda i: (0, jnp.minimum(i, NS - 1))),
            pl.BlockSpec((1, D), fixed),
            pl.BlockSpec((BS, D), p1),
            pl.BlockSpec((D, 3 * D), fixed),
            pl.BlockSpec((D, D), fixed),
            pl.BlockSpec((2 * C, C), fixed),
            pl.BlockSpec((C, 2 * C), fixed),
        ],
        out_specs=pl.BlockSpec((BS, 2 * D), p3),
        out_shape=jax.ShapeDtypeStruct((S, 2 * D), bf16),
        scratch_shapes=[
            pltpu.VMEM((D, D), bf16),
            pltpu.VMEM((4, S // 128, 128, 128), bf16),
            pltpu.VMEM((4, 2 + S // 128, 128, 128), bf16),
            pltpu.VMEM((2 + S // 128, 4, 256, 128), bf16),
            pltpu.VMEM((S // 128, 4, 128, 128), bf16),
            pltpu.VMEM((3, 128, 128), f32),
            pltpu.VMEM((8 + BS, D), f32),
            pltpu.VMEM((S, D), bf16),
            pltpu.VMEM((4, NC, 2 * C, 128), f32),
            pltpu.VMEM((4, NC, 2 * C, 128), f32),
            pltpu.VMEM((2 * C, D), f32),
            pltpu.VMEM((4, NC, 2 * C, 128), f32),
            pltpu.VMEM((4, 384, 128), f32),
            pltpu.VMEM((4, 8, 128), f32),
            pltpu.VMEM((4, 384, 128), f32),
            pltpu.VMEM((4, 8, 128), f32),
        ],
        compiler_params=pltpu.CompilerParams(
            dimension_semantics=("arbitrary",),
            vmem_limit_bytes=100 * 1024 * 1024,
        ),
    )(A_q[0], A_k[0], A_v[0], A_shift_k.T, A_ssm_k, A_ssm_D.reshape(1, D),
      B_x[0], B_wqkv, B_wo, jnp.asarray(fwd, bf16), jnp.asarray(inv, bf16))
    return out[None]
```
